```python
import os as _os
_os.environ.setdefault('JAX_PLATFORMS', 'cpu')
import jax
import jax.numpy as jnp

def _softmax(x, axis=-1):
    return jax.nn.softmax(x, axis=axis)

def _gelu(x):
    return jax.nn.gelu(x, approximate=True)

def _silu(x):
    return jax.nn.silu(x)

def _sigmoid(x):
    return jax.nn.sigmoid(x)

def _layernorm(x, axis=-1, eps=1e-05):
    m = jnp.mean(x, axis=axis, keepdims=True)
    v = jnp.var(x, axis=axis, keepdims=True)
    return (x - m) / jnp.sqrt(v + eps)

def _scatter_add(tgt, idx, src, axis=0):
    return tgt.at[idx].add(src)

def _segment_sum(src, seg, n):
    return jax.ops.segment_sum(src, seg, n)

class _Rng:

    def __init__(self, key):
        self._k = key

    def _next(self):
        self._k, sub = jax.random.split(self._k)
        return sub

    def normal(self, shape):
        return jax.random.normal(self._next(), shape, dtype=jnp.bfloat16)

    def randint(self, lo, hi, shape):
        return jax.random.randint(self._next(), shape, lo, hi, dtype=jnp.int32)

    def uniform(self, shape, lo=0.0, hi=1.0):
        return jax.random.uniform(self._next(), shape, jnp.bfloat16, lo, hi)

    def permutation(self, n):
        return jax.random.permutation(self._next(), n)
kernel_name = 'standalone__conformer_conv_module__speech'

def setup_inputs():
    _rng = _Rng(jax.random.key(int.from_bytes(__import__("os").urandom(4), "little")))
    _w = lambda a: (lambda t: t.astype(jnp.bfloat16) if jnp.issubdtype(t.dtype, jnp.floating) else t)(jnp.asarray(a))
    B, T, D, K = (2, 16000, 256, 5)
    return {'x': _w((lambda *s: _rng.normal(s) * 0.2)(B, T, D)), 'w_pw1': _w((lambda *s: _rng.normal(s) * 0.2)(D, 2 * D)), 'dw': _w((lambda *s: _rng.normal(s) * 0.05)(K, D)), 'w_pw2': _w((lambda *s: _rng.normal(s) * 0.05)(D, D))}

def reference(x, w_pw1, dw, w_pw2):
    B, T, D = x.shape
    K = dw.shape[0]
    h = x @ w_pw1
    a, b = (h[..., :D].copy(), h[..., D:].copy())
    h = a * _sigmoid(b)
    pad = K // 2
    hp = jnp.pad(h, ((0, 0), (pad, pad), (0, 0)))
    out = jnp.zeros_like(h)
    for i in range(K):
        out = out + hp[:, i:i + T, :] * dw[i][None, None, :]
    return _silu(out) @ w_pw2
```

```python
import functools

import jax
import jax.numpy as jnp
import jax.experimental.pallas as pl
import jax.experimental.pallas.tpu as pltpu

R = 320
WAITS = (0, 2, 5, 12, 28, 66)
INIT = 2
SECOND = 5
PACE = 4
OUT_START = 28
OUT_PACE = 2
GAP = 8
ORDER = "AAABAABBPBPBBPPPPPAAPB"
A_PRODUCTS = "1245367"
B_PRODUCTS = "2435167"
NP = 2

F32 = jnp.float32
BF16 = jnp.bfloat16
L = 128

_RESULTS = {
    (0, 0): ((1, 1), (4, 1), (5, -1), (7, 1)),
    (0, 1): ((3, 1), (5, 1)),
    (1, 0): ((2, 1), (4, 1)),
    (1, 1): ((1, 1), (2, -1), (3, 1), (6, 1)),
}


def _rhs_operands(b11, b12, b21, b22):
    ops = [b11 + b22, b11, b12 - b22, b21 - b11, b22, b11 + b12, b21 + b22]
    return [o.astype(BF16) for o in ops]


def _lhs_operand(i, a11, a12, a21, a22):
    return {1: lambda: a11 + a22, 2: lambda: a21 + a22, 3: lambda: a11, 4: lambda: a22,
            5: lambda: a11 + a12, 6: lambda: a21 - a11, 7: lambda: a12 - a22}[i]()


def _strassen_steps(order, lhs, rhs, emit):
    m = {}
    done = set()
    for ch in order:
        i = int(ch)
        m[i] = jnp.dot(lhs(i).astype(BF16), rhs[i - 1], preferred_element_type=F32)
        for c, terms in _RESULTS.items():
            if c not in done and all(t in m for t, _ in terms):
                done.add(c)
                ts = sorted(terms, key=lambda t: order.index(str(t[0])))
                if ts[0][1] < 0:
                    ts[0], ts[1] = ts[1], ts[0]
                acc = m[ts[0][0]]
                for t, sign in ts[1:]:
                    acc = acc + m[t] if sign > 0 else acc - m[t]
                emit(c, acc)
        yield


def _kernel(x_hbm, w1_hbm, dw_hbm, w2_hbm, o_hbm, x_v, o_v, h_v, w1_v, dw_v, w2_v,
            in_sems, w_sems, out_sem, *, T):
    rows = x_hbm.shape[0]
    K = dw_hbm.shape[0]
    pad = K // 2
    NC = rows // R
    H = R // 2
    chunks_per_seq = T // R
    bounds = list(WAITS) + [NC]
    group_of = [max(i for i in range(len(WAITS)) if bounds[i] <= g) for g in range(NC)]

    def x_rows(lo, hi, sem):
        return pltpu.make_async_copy(x_hbm.at[pl.ds(lo, hi - lo)], x_v.at[pl.ds(lo, hi - lo)], sem)

    issued = [0]
    waited = [0]

    def issue_x(upto):
        while issued[0] < min(upto, NC):
            g = issued[0]
            x_rows(g * R, (g + 1) * R, in_sems.at[group_of[g]]).start()
            issued[0] += 1

    def need_x(g):
        while waited[0] < len(WAITS) and bounds[waited[0]] <= g:
            s = waited[0]
            issue_x(bounds[s + 1])
            x_rows(bounds[s] * R, bounds[s + 1] * R, in_sems.at[s]).wait()
            waited[0] += 1

    sent = [0]

    def send_out(upto):
        while sent[0] < upto:
            sl = pl.ds(sent[0] * R, R)
            pltpu.make_async_copy(o_v.at[sl], o_hbm.at[sl], out_sem).start()
            sent[0] += 1

    w1_cp = pltpu.make_async_copy(w1_hbm, w1_v, w_sems.at[0])
    dw_cp = pltpu.make_async_copy(dw_hbm, dw_v, w_sems.at[1])
    w2_cp = pltpu.make_async_copy(w2_hbm, w2_v, w_sems.at[2])
    w1_cp.start()
    issue_x(INIT)
    dw_cp.start()

    n_seq = rows // T
    for b in range(n_seq + 1):
        lo = max(b * (T + 2 * GAP) - GAP, 0)
        hi = min(b * (T + 2 * GAP) + GAP, n_seq * (T + 2 * GAP))
        for j in range(2):
            h_v[j, pl.ds(lo, hi - lo), :] = jnp.zeros((hi - lo, L), F32)

    def h_row(g):
        return g * R + (g // chunks_per_seq) * (2 * GAP) + GAP

    w1_ops, w2_ops, s_vals = [], [], {}

    def a_plain(g):
        w = jnp.concatenate([w1_v[:, 0:L], w1_v[:, 2 * L:3 * L], w1_v[:, L:2 * L], w1_v[:, 3 * L:4 * L]], axis=1)
        ab = jnp.dot(x_v[pl.ds(g * R, R), :], w, preferred_element_type=F32)
        for j in range(2):
            a, b = ab[:, 2 * j * L:(2 * j + 1) * L], ab[:, (2 * j + 1) * L:(2 * j + 2) * L]
            h_v[j, pl.ds(h_row(g), R), :] = a * (jnp.tanh(b * 0.5) + 1.0)
        while True:
            yield

    def a_steps(g):
        xs = [x_v[pl.ds(g * R + r * H, H), c * L:(c + 1) * L] for r in range(2) for c in range(2)]
        fs = [v.astype(F32) for v in xs]

        def emit(c, v):
            h_v[c[1], pl.ds(h_row(g) + c[0] * H, H), :] = v[:, :L] * (jnp.tanh(v[:, L:]) + 1.0)

        lhs = lambda i: _lhs_operand(i, *(xs if i in (3, 4) else fs))
        return _strassen_steps(A_PRODUCTS, lhs, w1_ops, emit)

    def p_steps(g):
        dw = dw_v[...].astype(F32) * 0.25
        n = H // NP
        pieces = [(i, p) for p in range(NP) for i in range(4) if not (i >= 2 and p == NP - 1)]
        for i, p in pieces + [(3, NP - 1), (2, NP - 1)]:
            r, j = divmod(i, 2)
            y = None
            for k in range(K):
                t = h_v[j, pl.ds(h_row(g) + r * H + p * n + (k - pad), n), :] * dw[k:k + 1, j * L:(j + 1) * L]
                y = t if y is None else y + t
            s_vals[(g, i, p)] = y * (jnp.tanh(y) + 1.0)
            yield

    def b_steps(g):
        def quadrant(i):
            return jnp.concatenate([s_vals[(g, i, p)] for p in range(NP)], axis=0)

        def lhs(i):
            need = {1: (0, 3), 2: (2, 3), 3: (0,), 4: (3,), 5: (0, 1), 6: (2, 0), 7: (1, 3)}[i]
            q = {k: quadrant(k) for k in need}
            return _lhs_operand(i, *[q.get(k) for k in range(4)])

        def emit(c, v):
            o_v[pl.ds(g * R + c[0] * H, H), c[1] * L:(c[1] + 1) * L] = v.astype(o_v.dtype)

        return _strassen_steps(B_PRODUCTS, lhs, w2_ops, emit)

    w1_cp.wait()
    w2_cp.start()
    issue_x(SECOND)
    need_x(0)
    dw_cp.wait()
    for g in range(-2, NC):
        if g >= -1:
            issue_x(SECOND + PACE * (g + 1))
        if g + 2 < NC:
            need_x(g + 2)
        if g == -2:
            w1 = w1_v[...].astype(F32)
            n1 = jnp.concatenate([w1[:, 0:L], w1[:, 2 * L:3 * L] * 0.5], axis=1)
            n2 = jnp.concatenate([w1[:, L:2 * L], w1[:, 3 * L:4 * L] * 0.5], axis=1)
            w1_ops.extend(_rhs_operands(n1[:L], n2[:L], n1[L:], n2[L:]))
        if g == 0:
            w2_cp.wait()
            w2 = w2_v[...].astype(F32)
            w2_ops.extend(_rhs_operands(w2[:L, :L], w2[:L, L:], w2[L:, :L], w2[L:, L:]))
        stages = {
            "A": (a_plain if g == -2 else a_steps)(g + 2) if g + 2 < NC else None,
            "P": p_steps(g + 1) if 0 <= g + 1 < NC else None,
            "B": b_steps(g) if g >= 0 else None,
        }
        for t in ORDER:
            if stages[t] is not None:
                next(stages[t])
        if g >= OUT_START:
            send_out(min(g + 1, sent[0] + OUT_PACE))
    send_out(NC)
    pltpu.make_async_copy(o_v, o_hbm, out_sem).wait()


@jax.jit
def pallas_standalone__conformer_conv_module__speech_kernel(x, w_pw1, dw, w_pw2):
    B, T, D = x.shape
    K = dw.shape[0]
    rows = B * T
    assert D == 2 * L and T % R == 0 and K // 2 <= GAP and rows // R > WAITS[-1]
    any_spec = pl.BlockSpec(memory_space=pl.ANY)
    out = pl.pallas_call(
        functools.partial(_kernel, T=T),
        in_specs=[any_spec] * 4,
        out_specs=any_spec,
        out_shape=jax.ShapeDtypeStruct((rows, D), x.dtype),
        scratch_shapes=[
            pltpu.VMEM((rows, D), x.dtype),
            pltpu.VMEM((rows, D), x.dtype),
            pltpu.VMEM((2, B * (T + 2 * GAP), L), F32),
            pltpu.VMEM((D, 2 * D), w_pw1.dtype),
            pltpu.VMEM((K, D), dw.dtype),
            pltpu.VMEM((D, D), w_pw2.dtype),
            pltpu.SemaphoreType.DMA((len(WAITS),)),
            pltpu.SemaphoreType.DMA((3,)),
            pltpu.SemaphoreType.DMA(()),
        ],
        compiler_params=pltpu.CompilerParams(vmem_limit_bytes=110 * 1024 * 1024),
    )(x.reshape(rows, D), w_pw1, dw, w_pw2)
    return out.reshape(B, T, D)
```
